```python
import os as _os
_os.environ.setdefault("JAX_PLATFORMS", "cpu")
import jax
import jax.numpy as jnp

def _softmax(x, axis=-1):
    return jax.nn.softmax(x, axis=axis)
def _gelu(x):
    return jax.nn.gelu(x, approximate=True)
def _silu(x):
    return jax.nn.silu(x)
def _sigmoid(x):
    return jax.nn.sigmoid(x)
def _layernorm(x, axis=-1, eps=1e-5):
    m = jnp.mean(x, axis=axis, keepdims=True)
    v = jnp.var(x, axis=axis, keepdims=True)
    return (x - m) / jnp.sqrt(v + eps)
def _scatter_add(tgt, idx, src, axis=0):
    return tgt.at[idx].add(src)
def _segment_sum(src, seg, n):
    return jax.ops.segment_sum(src, seg, n)
class _Rng:
    def __init__(self, key):
        self._k = key
    def _next(self):
        self._k, sub = jax.random.split(self._k)
        return sub
    def normal(self, shape):
        return jax.random.normal(self._next(), shape, dtype=jnp.bfloat16)
    def randint(self, lo, hi, shape):
        return jax.random.randint(self._next(), shape, lo, hi, dtype=jnp.int32)
    def uniform(self, shape, lo=0.0, hi=1.0):
        return jax.random.uniform(self._next(), shape, jnp.bfloat16, lo, hi)
    def permutation(self, n):
        return jax.random.permutation(self._next(), n)


kernel_name = 'interleave_layers__linear_kernel_hedgehog__ssm_conv_s4__prompt'

def setup_inputs():
    _rng = _Rng(jax.random.key(int.from_bytes(__import__("os").urandom(4), "little")))
    _w = (lambda a: (lambda t: t.astype(jnp.bfloat16) if jnp.issubdtype(t.dtype, jnp.floating) else t)(jnp.asarray(a)))
    def _A_setup():
        B, S, D, H = 1, 2048, 512, 32
        Dh = D // H
        return {
            "x": _w((lambda *s: _rng.normal(s) * 0.05)(B, S, D)),
            "wqkv": _w((lambda *s: _rng.normal(s) * 0.4)(D, 3 * D)),
            "w_phi": _w((lambda *s: _rng.normal(s) * 0.4)(H, Dh, Dh) * (Dh ** -0.5)),
            "wo": _w((lambda *s: _rng.normal(s) * 0.05)(D, D)),
        }
    _A_in = _A_setup()

    def _B_setup():
        B, L, D, N = 1, 2048, 512, 128
        A_re = -jnp.exp((lambda *s: _rng.normal(s) * 0.2)(D, N))
        A_im = jnp.pi * (lambda *s: _rng.normal(s) * 0.2)(D, N)
        B_re = (lambda *s: _rng.normal(s) * 0.2)(D, N)
        B_im = (lambda *s: _rng.normal(s) * 0.2)(D, N)
        C_re = (lambda *s: _rng.normal(s) * 0.2)(D, N)
        C_im = (lambda *s: _rng.normal(s) * 0.2)(D, N)
        log_dt = (lambda *s: _rng.normal(s) * 0.2)(D) * 0.5 - 4.0
        Dskip = (lambda *s: _rng.normal(s) * 0.2)(D)
        return {
            "u": _w((lambda *s: _rng.normal(s) * 0.05)(B, L, D)),
            "A_re": _w(A_re),
            "A_im": _w(A_im),
            "B_re": _w(B_re),
            "B_im": _w(B_im),
            "C_re": _w(C_re),
            "C_im": _w(C_im),
            "log_dt": _w(log_dt),
            "Dskip": _w(Dskip),
        }
    _B_in = _B_setup()

    return {
        "A_x": _A_in["x"],
        "A_wqkv": _A_in["wqkv"],
        "A_w_phi": _A_in["w_phi"],
        "A_wo": _A_in["wo"],
        "B_u": _B_in["u"],
        "B_A_re": _B_in["A_re"],
        "B_A_im": _B_in["A_im"],
        "B_B_re": _B_in["B_re"],
        "B_B_im": _B_in["B_im"],
        "B_C_re": _B_in["C_re"],
        "B_C_im": _B_in["C_im"],
        "B_log_dt": _B_in["log_dt"],
        "B_Dskip": _B_in["Dskip"],
    }

def reference(A_x, A_wqkv, A_w_phi, A_wo, B_u, B_A_re, B_A_im, B_B_re, B_B_im, B_C_re, B_C_im, B_log_dt, B_Dskip):
    def _A_ref(x, wqkv, w_phi, wo):
        B, S, D = x.shape
        H = 32; Dh = D // H
        qkv = (lambda x, *d: x.transpose(*d))((x @ wqkv).reshape(B, S, 3, H, Dh), 2, 0, 3, 1, 4)
        q, k, v = qkv[0], qkv[1], qkv[2]
        pq = jnp.einsum("bhsd,hdf->bhsf", q, w_phi)
        pk = jnp.einsum("bhsd,hdf->bhsf", k, w_phi)
        phi_q = jnp.concatenate([_softmax(pq, axis=-1), _softmax(-pq, axis=-1)], axis=-1)
        phi_k = jnp.concatenate([_softmax(pk, axis=-1), _softmax(-pk, axis=-1)], axis=-1)
        kv = jnp.einsum("bhsf,bhsd->bhfd", phi_k, v)
        z  = jnp.einsum("bhsf->bhf", phi_k)
        num = jnp.einsum("bhqf,bhfd->bhqd", phi_q, kv)
        den = jnp.einsum("bhqf,bhf->bhq", phi_q, z)[..., None] + 1e-6
        o = num / den
        return (lambda x, *d: x.transpose(*d))(o, 0, 2, 1, 3).reshape(B, S, D) @ wo

    def _B_ref(u, A_re, A_im, B_re, B_im, C_re, C_im, log_dt, Dskip):
        Bsz, L, D = u.shape
        dt = jnp.exp(log_dt)[:, None]
        A = A_re + 1j * A_im
        Bc = B_re + 1j * B_im
        Cc = C_re + 1j * C_im
        logdA = dt * A
        dB = dt * Bc
        l = (lambda x, dt: x.astype(dt))(jnp.arange(L), A_re.dtype)
        P = jnp.exp(logdA[:, :, None] * l[None, None, :])
        K = jnp.einsum("dn,dnl,dn->dl", Cc, P, dB).real
        L2 = 2 * L
        Kp = jnp.pad(K, ((0, 0), (0, L)))
        up = (lambda x, *d: x.transpose(*d))(u, 0, 2, 1)
        up = jnp.pad(up, ((0, 0), (0, 0), (0, L)))
        Kf = (lambda x, axes=(-2,-1): jnp.fft.rfft2(x.astype(jnp.float32), axes=axes))(Kp[:, None, :], axes=(-2, -1))
        Uf = (lambda x, axes=(-2,-1): jnp.fft.rfft2(x.astype(jnp.float32), axes=axes))(up[:, :, None, :], axes=(-2, -1))
        Yf = Uf * Kf[None, :, :, :]
        y = (lambda x, s, axes=(-2,-1): jnp.fft.irfft2(x, s=s, axes=axes).astype(jnp.bfloat16))(Yf, (1, L2), axes=(-2, -1))[:, :, 0, :L]
        y = (lambda x, *d: x.transpose(*d))(y, 0, 2, 1) + u * Dskip[None, None, :]
        return y

    x = A_x
    x = x + _A_ref(_layernorm(x, axis=-1), A_wqkv, A_w_phi, A_wo)
    x = x + _B_ref(_layernorm(x, axis=-1), B_A_re, B_A_im, B_B_re, B_B_im, B_C_re, B_C_im, B_log_dt, B_Dskip)
    x = x + _A_ref(_layernorm(x, axis=-1), A_wqkv, A_w_phi, A_wo)
    x = x + _B_ref(_layernorm(x, axis=-1), B_A_re, B_A_im, B_B_re, B_B_im, B_C_re, B_C_im, B_log_dt, B_Dskip)
    return x
```

```python
import numpy as np
import ml_dtypes
import jax
import jax.numpy as jnp
from jax import lax
import jax.experimental.pallas as pl
import jax.experimental.pallas.tpu as pltpu

S, D, H, DH, N = 2048, 512, 32, 16, 128
F32, BF16, U32 = jnp.float32, jnp.bfloat16, jnp.uint32
NN = (((1,), (0,)), ((), ()))
NT = (((1,), (1,)), ((), ()))
TN = (((0,), (0,)), ((), ()))
LOG2E = 1.4426950408889634
CS = 256
KU = 64
GC, TC = 4, 2
KP, KTP, VP, P1, P2, PX = 36, 20, 12, 132, 20, 17


def _fft_constants():
    f1 = np.arange(128)
    th = 2 * np.pi * np.outer(f1 + 0.5, f1) / 256
    w1 = np.stack([np.cos(th), -np.sin(th)], 1).reshape(256, 128)
    w1i = np.stack([np.cos(th).T, -np.sin(th).T], -1).reshape(128, 256)
    a = np.arange(16)
    m2f = np.zeros((32, 2, 4, 16, 4, 16, 2))
    m2i = np.zeros((32, 4, 16, 2, 2, 4, 16))
    for g in range(32):
        for s in range(4):
            t = 2 * np.pi * (np.outer(a, a) / 16 + (4 * g + s + 0.5) * a[None, :] / 4096)
            c, sn = np.cos(t), np.sin(t)
            m2f[g, 0, s, :, s, :, 0] = c
            m2f[g, 0, s, :, s, :, 1] = sn
            m2f[g, 1, s, :, s, :, 0] = -sn
            m2f[g, 1, s, :, s, :, 1] = c
            m2i[g, s, :, 0, 0, s, :] = c.T
            m2i[g, s, :, 0, 1, s, :] = -sn.T
            m2i[g, s, :, 1, 0, s, :] = sn.T
            m2i[g, s, :, 1, 1, s, :] = c.T
    cast = lambda v: np.asarray(v, np.float32).astype(ml_dtypes.bfloat16)
    return cast(w1), cast(w1i), cast(m2f.reshape(32, 128, 128)), cast(m2i.reshape(32, 128, 128))


def _lag_rounding():
    l = np.arange(S)
    rl = l.astype(np.float32).astype(ml_dtypes.bfloat16).astype(np.float32).astype(np.int64)
    r = (rl - 16 * (l // 16)).reshape(128, 16)
    return [[int(v) for v in r[t1]] for t1 in (0, 16, 32, 64)]


def _dot(a, b, dn=NN):
    return lax.dot_general(a, b, dn, preferred_element_type=F32)


def _cmul(ar, ai, br, bi):
    return ar * br - ai * bi, ar * bi + ai * br


def _layernorm(x):
    m = jnp.mean(x, axis=-1, keepdims=True)
    c = x - m
    v = jnp.mean(c * c, axis=-1, keepdims=True)
    return c * lax.rsqrt(v + 1e-5)


def _pair(v, op):
    return op(v, pltpu.roll(v, 4, 0))


def _dual_softmax(p):
    s = p.shape[-1]
    p3 = p.reshape(8, 8, s)
    ep = jnp.exp2(p3 - _pair(jnp.max(p3, axis=0), jnp.maximum))
    en = jnp.exp2(_pair(jnp.min(p3, axis=0), jnp.minimum) - p3)
    ep = ep * (1.0 / _pair(jnp.sum(ep, axis=0), jnp.add))
    en = en * (1.0 / _pair(jnp.sum(en, axis=0), jnp.add))
    return jnp.concatenate([ep.reshape(64, s), en.reshape(64, s)], axis=0)


def _pack(y):
    return pltpu.bitcast(y.astype(BF16), U32)


def _kernel(x_hbm, wqkv_hbm, wphi_ref, wo_hbm, are_hbm, aim_hbm, bre_hbm, bim_hbm, cre_hbm, cim_hbm,
            ldt_ref, dsk_ref, w1_hbm, w1i_hbm, m2f_hbm, m2i_hbm, o_hbm,
            x_ref, wqkv_ref, wo_ref, par, w1_ref, w1i_ref, m2f_ref, m2i_ref, o_ref, sems, osems,
            xs, nat, xn, wt, wop, kf, sh, sh2, kt, ft, vt, gt, kv_s, z_s, lb0, lb1, kvt,
            pb0, pb1, vb0, vb1, fb0, fb1, gb0, gb1):
    fbuf, gbuf, lbuf = (fb0, fb1), (gb0, gb1), (lb0, lb1)
    pbuf, vbuf = (pb0, pb1), (vb0, vb1)
    seg = _lag_rounding()
    row = lax.broadcasted_iota(jnp.int32, (128, 128), 0)
    col = lax.broadcasted_iota(jnp.int32, (128, 128), 1)

    pairs = [(h, par.at[i]) for i, h in enumerate((are_hbm, aim_hbm, bre_hbm, bim_hbm, cre_hbm, cim_hbm))]
    pairs += [(w1_hbm, w1_ref), (m2f_hbm, m2f_ref), (wqkv_hbm, wqkv_ref), (wo_hbm, wo_ref), (x_hbm, x_ref),
              (m2i_hbm, m2i_ref), (w1i_hbm, w1i_ref)]
    copies = [pltpu.make_async_copy(a, b, sems.at[i]) for i, (a, b) in enumerate(pairs)]
    for cp in copies:
        cp.start()
    for cp in copies[:6]:
        cp.wait()
    are_ref, aim_ref, bre_ref, bim_ref, cre_ref, cim_ref = (par.at[i] for i in range(6))

    dt = jnp.exp(ldt_ref[...].astype(F32).reshape(1, D)).astype(BF16).astype(F32)
    dtc = jnp.broadcast_to(dt, (128, D)).T
    ar, ai = dtc * are_ref[...].astype(F32), dtc * aim_ref[...].astype(F32)
    mag = jnp.exp(ar)
    pr, pi = mag * jnp.cos(ai), mag * jnp.sin(ai)
    cr, ci = _cmul(cre_ref[...].astype(F32), cim_ref[...].astype(F32),
                   dtc * bre_ref[...].astype(F32), dtc * bim_ref[...].astype(F32))
    sq = lambda r, i_: (r * r - i_ * i_, 2.0 * r * i_)
    kend = []
    for c in range(4):
        rows = slice(128 * c, 128 * c + 128)
        qr, qi = pr[rows], pi[rows]
        q16 = (qr, qi)
        for _ in range(4):
            q16 = sq(*q16)
        er, ei = jnp.ones((128, 128), F32), jnp.zeros((128, 128), F32)
        for i in range(8):
            r = pl.ds(128 * c * VP + i, 128, stride=VP)
            vt[0, r, :], vt[1, r, :] = er, ei
            er, ei = _cmul(er, ei, *q16) if i else q16
        gt[0, rows, :], gt[1, rows, :] = er, ei
        half = sq(*sq(*sq(er, ei)))
        f0 = (cr[rows], ci[rows])
        f1 = _cmul(*f0, *half)
        tail = _cmul(*f1, *half)
        kend.append(jnp.sum(tail[0], axis=-1, keepdims=True))
        for i in range(16):
            for a, f in enumerate((f0, f1)):
                r = pl.ds(128 * c * KP + 16 * a + i, 128, stride=KP)
                ft[0, r, :], ft[1, r, :] = f
            if i < 15:
                f0, f1 = _cmul(*f0, qr, qi), _cmul(*f1, qr, qi)

    low = lax.broadcasted_iota(jnp.int32, (16, 128), 1) < 64

    def kgen(i, carry):
        for u in range(KU):
            d = i * KU + u
            gr = jnp.broadcast_to(gt[0, pl.ds(d, 1), :], (8, 128))
            gi = jnp.broadcast_to(gt[1, pl.ds(d, 1), :], (8, 128))
            rv = pl.ds(pl.multiple_of(d * VP, 4), 8)
            es = [(vt[0, rv, :], vt[1, rv, :])]
            for _ in range(7):
                es.append(_cmul(*es[-1], gr, gi))
            e = jnp.concatenate([v[0] for v in es] + [v[1] for v in es], axis=0).astype(BF16)
            rf = pl.ds(pl.multiple_of(d * KP, 4), 32)
            o = _dot(jnp.concatenate([ft[0, rf, :], ft[1, rf, :]], axis=0).astype(BF16), e, NT)
            swap = lambda v: pltpu.roll(v, 64, 1)
            k = jnp.where(low, o[0:16], swap(o[16:32])) - jnp.where(low, swap(o[32:48]), o[48:64])
            kt[pl.ds(pl.multiple_of(d * KTP, 4), 16), :] = k
        return carry
    lax.fori_loop(0, D // KU, kgen, 0)

    def stage2_fwd(g):
        z = jnp.concatenate(
            [jnp.concatenate([sh[j, pl.ds(g * 4 + s, 16, stride=P1), :] for s in range(4)], axis=0)
             for j in range(4)], axis=1)
        return _dot(m2f_ref[g], pltpu.bitcast(z, BF16))

    kend_t = [jnp.where(col == 127, kend[c], pltpu.roll(kt[pl.ds(c * 128 * KTP, 128, stride=KTP), :], 127, 1))
              for c in range(4)]
    copies[6].wait()
    copies[7].wait()
    copies[10].wait()
    for t2 in range(16):
        for dtile in range(4):
            def ldk(i):
                if i < 16:
                    return kt[pl.ds(dtile * 128 * KTP + i, 128, stride=KTP), :]
                return kend_t[dtile]
            k = jnp.where(col < 16, ldk(seg[0][t2]),
                          jnp.where(col < 32, ldk(seg[1][t2]), jnp.where(col < 64, ldk(seg[2][t2]), ldk(seg[3][t2]))))
            y = _dot(w1_ref[...], k.astype(BF16), NT)
            sh[dtile, t2 * P1:t2 * P1 + 128, :] = _pack(y)
        xv = x_ref[128 * t2:128 * t2 + 128, :].astype(F32)
        for q in range(8):
            for j in range(4):
                nat[j, (8 * t2 + q) * PX:(8 * t2 + q) * PX + 16, :] = xv[16 * q:16 * q + 16, 128 * j:128 * j + 128]
    dsk = dsk_ref[...].astype(F32).reshape(1, D)

    for t2 in range(16):
        for j in range(4):
            xs[t2 * 128:(t2 + 1) * 128, 128 * j:128 * j + 128] = nat[j, pl.ds(t2, 128, stride=PX), :]

    def kspec(i, carry):
        for u in range(8):
            g = i * 8 + u
            xf = stage2_fwd(g)
            kf[g, :64, :] = (xf[:64] + dsk) * (2.0 / 4096)
            kf[g, 64:, :] = xf[64:] * (2.0 / 4096)
        r = pl.ds(pl.multiple_of(i * (S // 4), S // 4), S // 4)
        xn[r, :] = _layernorm(xs[r, :]).astype(BF16)
        return carry
    lax.fori_loop(0, 4, kspec, 0)

    copies[8].wait()
    copies[9].wait()
    onehot = lambda m: jnp.where(m, 1.0, 0.0).astype(BF16)
    rep = onehot(lax.broadcasted_iota(jnp.int32, (128, 16), 0) % 64 // 4 == lax.broadcasted_iota(jnp.int32, (128, 16), 1))
    p2 = wphi_ref[...].reshape(256, 32)
    r256 = lax.broadcasted_iota(jnp.int32, (256, 128), 0)
    c256 = lax.broadcasted_iota(jnp.int32, (256, 128), 1)
    head = 4 * (row // 64) + row % 4
    perm = onehot(head * 16 + row % 64 // 4 == col)
    bdts = []
    for g in range(4):
        selh = onehot(lax.broadcasted_iota(jnp.int32, (32, 128), 0)
                      == 8 * g + lax.broadcasted_iota(jnp.int32, (32, 128), 1) // 16)
        b = jnp.where(r256 // 16 == c256 % 16, _dot(p2, selh), 0.0)
        b = jnp.sum(b.reshape(16, 16, 128), axis=0).astype(BF16)
        bdts.append(jnp.where(head == col // 16, _dot(rep, b), 0.0).astype(BF16))
    for g in range(4):
        cols = lambda j: wqkv_ref[:, j * D + 128 * g:j * D + 128 * g + 128]
        lhs = jnp.concatenate([bdts[g], bdts[g], perm], axis=0)
        for j in range(3):
            r = _dot(lhs[128 * j:128 * j + 128], cols(j), NT)
            wt[j * D + 128 * g:j * D + 128 * g + 128, :] = (r * LOG2E if j < 2 else r).astype(BF16)
        wop[128 * g:128 * g + 128, :] = _dot(perm, wo_ref[128 * g:128 * g + 128, :]).astype(BF16)

    def pipeline(stages, n):
        depth = len(stages) - 1
        def step(t, lo, hi, par):
            for k, fn in enumerate(stages):
                if lo <= t - k if isinstance(t, int) else True:
                    if not isinstance(t, int) or t - k < hi:
                        fn(t - k, (par - k) % 2)
        first = depth + (depth % 2)
        for t in range(first):
            step(t, 0, n, t % 2)
        def body(j, carry):
            step(first + 2 * j, 0, n, 0)
            step(first + 2 * j + 1, 0, n, 1)
            return carry
        lax.fori_loop(0, (n - first) // 2, body, 0)
        for t in range(n, n + depth):
            step(t, 0, n, t % 2)

    def rows(c):
        return pl.ds(c * CS if isinstance(c, int) else pl.multiple_of(c * CS, CS), CS)

    def attention():
        kv_s[...] = jnp.zeros(kv_s.shape, F32)
        z_s[...] = jnp.zeros(z_s.shape, F32)

        def proj_kv(c, b):
            res = _dot(wt[D:3 * D, :], xn[rows(c), :], NT)
            pbuf[b][...] = res[:D]
            vbuf[b][...] = res[D:].astype(BF16)

        def post_kv(c, b):
            for q in range(8):
                ph = _dual_softmax(pbuf[b][64 * q:64 * q + 64, :])
                zz = ph[:, :128]
                for j in range(1, CS // 128):
                    zz = zz + ph[:, 128 * j:128 * j + 128]
                z_s[q] += zz
                kv_s[q] += _dot(vbuf[b][64 * q:64 * q + 64, :], ph.astype(BF16), NT)
        pipeline([proj_kv, post_kv], S // CS)

        for q in range(8):
            kvt[q] = jnp.where(row[:64] % 4 == col[:64] % 4, kv_s[q], 0.0).astype(BF16)
            z_s[q] = jnp.broadcast_to(jnp.sum(z_s[q], axis=-1, keepdims=True), (128, 128))

        def proj_q(c, b):
            pbuf[b][...] = _dot(wt[0:D, :], xn[rows(c), :], NT)

        def post_q(c, b):
            for q in range(8):
                ph = _dual_softmax(pbuf[b][64 * q:64 * q + 64, :])
                pz = ph * jnp.concatenate([z_s[q]] * (CS // 128), axis=1)
                den = _pair(jnp.sum(pz.reshape(16, 8, CS), axis=0), jnp.add) + 1e-6
                num = _dot(kvt[q], ph.astype(BF16))
                o = num.reshape(8, 8, CS) * (1.0 / den)
                vbuf[b][64 * q:64 * q + 64, :] = o.reshape(64, CS).astype(BF16)

        def out_proj(c, b):
            r = rows(c)
            xnew = xs[r, :] + _dot(vbuf[b][...], wop[...], TN)
            xs[r, :] = xnew
            lbuf[b][...] = _layernorm(xnew).astype(BF16)

        def dft1(c, b):
            for u in range(CS // 128):
                t2 = c * (CS // 128) + u
                y = _dot(w1_ref[...], lbuf[b][128 * u:128 * u + 128, :])
                y = _pack(y)
                r1 = t2 * P1
                for j in range(4):
                    sh[j, pl.ds(r1 if isinstance(r1, int) else pl.multiple_of(r1, 4), 128), :] = y[:, 128 * j:128 * j + 128]
        pipeline([proj_q, post_q, out_proj, dft1], S // CS)

    def ssm_conv(l):
        def c2a(c, b):
            for u in range(GC):
                fbuf[b][128 * u:128 * u + 128, :] = stage2_fwd(c * GC + u)

        def c2b(c, b):
            for u in range(GC):
                g = c * GC + u
                xf = fbuf[b][128 * u:128 * u + 128, :]
                p_r, p_i = _cmul(xf[:64], xf[64:], kf[g, :64, :], kf[g, 64:, :])
                gbuf[b][128 * u:128 * u + 128, :] = jnp.concatenate([p_r, p_i], axis=0).astype(BF16)

        def c2c(c, b):
            for u in range(GC):
                g = c * GC + u
                q = _pack(_dot(m2i_ref[g], gbuf[b][128 * u:128 * u + 128, :]))
                for s in range(4):
                    r0 = (g * 4 + s) * P2
                    r = pl.ds(r0 if isinstance(r0, int) else pl.multiple_of(r0, 4), 16)
                    for j in range(4):
                        sh2[j, r, :] = q[16 * s:16 * s + 16, 128 * j:128 * j + 128]
        pipeline([c2a, c2b, c2c], 32 // GC)

        def c3a(c, b):
            for u in range(TC):
                q = jnp.concatenate([sh2[j, pl.ds(c * TC + u, 128, stride=P2), :] for j in range(4)], axis=1)
                fbuf[b][128 * u:128 * u + 128, :] = _dot(w1i_ref[...], pltpu.bitcast(q, BF16))

        def c3b(c, b):
            for u in range(TC):
                t2 = c * TC + u
                r = pl.ds(t2 * 128 if isinstance(t2, int) else pl.multiple_of(t2 * 128, 128), 128)
                xnew = xs[r, :] + fbuf[b][128 * u:128 * u + 128, :]
                xs[r, :] = xnew
                xn[r, :] = _layernorm(xnew).astype(BF16)

        def c3_last(c, b):
            for u in range(TC):
                t2 = c * TC + u
                q = jnp.concatenate([sh2[j, pl.ds(t2, 128, stride=P2), :] for j in range(4)], axis=1)
                r = pl.ds(pl.multiple_of(t2 * 128, 128), 128)
                xnew = xs[r, :] + _dot(w1i_ref[...], pltpu.bitcast(q, BF16))
                for j in range(4):
                    nat[j, pl.ds(t2, 128, stride=PX), :] = xnew[:, 128 * j:128 * j + 128]

        @pl.when(l == 0)
        def _():
            pipeline([c3a, c3b], 16 // TC)

        @pl.when(l == 1)
        def _():
            pipeline([c3_last], 16 // TC)

    copies[11].wait()
    copies[12].wait()

    def layer(l, carry):
        attention()
        ssm_conv(l)
        return carry
    lax.fori_loop(0, 2, layer, 0)

    ops = []
    for c in range(S // CS):
        for q in range(CS // 16):
            t1 = c * (CS // 16) + q
            blk = jnp.concatenate([nat[j, pl.ds(t1 * PX, 16), :] for j in range(4)], axis=1)
            o_ref[t1 * 16:t1 * 16 + 16, :] = blk.astype(o_ref.dtype)
        ops.append(pltpu.make_async_copy(o_ref.at[c * CS:(c + 1) * CS, :], o_hbm.at[c * CS:(c + 1) * CS, :], osems.at[c]))
        ops[-1].start()
    for cp in ops:
        cp.wait()


def _call(x, wqkv, wphi, wo, are, aim, bre, bim, cre, cim, ldt, dsk, interpret=False):
    consts = _fft_constants()
    hbm, vmem = pl.BlockSpec(memory_space=pl.ANY), pl.BlockSpec(memory_space=pltpu.VMEM)
    return pl.pallas_call(
        _kernel,
        out_shape=jax.ShapeDtypeStruct((S, D), x.dtype),
        in_specs=[hbm, hbm, vmem, hbm] + [hbm] * 6 + [vmem, vmem] + [hbm] * 4,
        out_specs=hbm,
        scratch_shapes=[
            pltpu.VMEM((S, D), BF16),
            pltpu.VMEM((D, 3 * D), BF16),
            pltpu.VMEM((D, D), BF16),
            pltpu.VMEM((6, D, N), BF16),
            pltpu.VMEM((256, 128), BF16),
            pltpu.VMEM((128, 256), BF16),
            pltpu.VMEM((32, 128, 128), BF16),
            pltpu.VMEM((32, 128, 128), BF16),
            pltpu.VMEM((S, D), BF16),
            pltpu.SemaphoreType.DMA((13,)),
            pltpu.SemaphoreType.DMA((S // CS,)),
            pltpu.VMEM((S, D), F32),
            pltpu.VMEM((4, 129 * PX + 7, 128), F32),
            pltpu.VMEM((S, D), BF16),
            pltpu.VMEM((3 * D, D), BF16),
            pltpu.VMEM((D, D), BF16),
            pltpu.VMEM((32, 128, D), F32),
            pltpu.VMEM((4, 17 * P1 + 4, 128), U32),
            pltpu.VMEM((4, 130 * P2, 128), U32),
            pltpu.VMEM(((D + 2) * KTP, 128), F32),
            pltpu.VMEM((2, (D + 2) * KP, 128), F32),
            pltpu.VMEM((2, (D + 2) * VP, 128), F32),
            pltpu.VMEM((2, D, 128), F32),
            pltpu.VMEM((8, 64, 128), F32),
            pltpu.VMEM((8, 128, 128), F32),
            pltpu.VMEM((CS, D), BF16),
            pltpu.VMEM((CS, D), BF16),
            pltpu.VMEM((8, 64, 128), BF16),
            pltpu.VMEM((D, CS), F32),
            pltpu.VMEM((D, CS), F32),
            pltpu.VMEM((D, CS), BF16),
            pltpu.VMEM((D, CS), BF16),
            pltpu.VMEM((128 * max(GC, TC), D), F32),
            pltpu.VMEM((128 * max(GC, TC), D), F32),
            pltpu.VMEM((128 * GC, D), BF16),
            pltpu.VMEM((128 * GC, D), BF16),
        ],
        compiler_params=pltpu.CompilerParams(vmem_limit_bytes=100 * 1024 * 1024),
        interpret=interpret,
    )(x, wqkv, wphi, wo, are, aim, bre, bim, cre, cim, ldt, dsk, *consts)


@jax.jit
def pallas_interleave_layers__linear_kernel_hedgehog__ssm_conv_s4__prompt_kernel(
    A_x: jax.Array,
    A_wqkv: jax.Array,
    A_w_phi: jax.Array,
    A_wo: jax.Array,
    B_u: jax.Array,
    B_A_re: jax.Array,
    B_A_im: jax.Array,
    B_B_re: jax.Array,
    B_B_im: jax.Array,
    B_C_re: jax.Array,
    B_C_im: jax.Array,
    B_log_dt: jax.Array,
    B_Dskip: jax.Array,
):
    del B_u
    out = _call(A_x.reshape(S, D), A_wqkv, A_w_phi.transpose(1, 2, 0), A_wo, B_A_re, B_A_im, B_B_re, B_B_im, B_C_re, B_C_im,
                B_log_dt, B_Dskip)
    return out.reshape(1, S, D)
```
